```python
import jax
import jax.numpy as jnp

def _softmax(x, axis=-1):
    return jax.nn.softmax(x, axis=axis)
def _gelu(x):
    return jax.nn.gelu(x, approximate=True)
def _silu(x):
    return jax.nn.silu(x)
def _sigmoid(x):
    return jax.nn.sigmoid(x)
def _layernorm(x, axis=-1, eps=1e-5):
    m = jnp.mean(x, axis=axis, keepdims=True)
    v = jnp.var(x, axis=axis, keepdims=True)
    return (x - m) / jnp.sqrt(v + eps)
def _scatter_add(tgt, idx, src, axis=0):
    return tgt.at[idx].add(src)
def _segment_sum(src, seg, n):
    return jax.ops.segment_sum(src, seg, n)
class _Rng:
    def __init__(self, key):
        self._k = key
    def _next(self):
        self._k, sub = jax.random.split(self._k)
        return sub
    def normal(self, shape):
        return jax.random.normal(self._next(), shape, dtype=jnp.bfloat16)
    def randint(self, lo, hi, shape):
        return jax.random.randint(self._next(), shape, lo, hi, dtype=jnp.int32)
    def uniform(self, shape, lo=0.0, hi=1.0):
        return jax.random.uniform(self._next(), shape, jnp.bfloat16, lo, hi)
    def permutation(self, n):
        return jax.random.permutation(self._next(), n)


kernel_name = 'sequential_preLN__sliding_block_cached__glu_gated_swiglu__decode'

def setup_inputs():
    _rng = _Rng(jax.random.key(int.from_bytes(__import__("os").urandom(4), "little")))
    _w = (lambda a: (lambda t: t.astype(jnp.bfloat16) if jnp.issubdtype(t.dtype, jnp.floating) else t)(jnp.asarray(a)))
    def _A_setup():
        B, Sq, D = 1, 1, 640
        Hq, Hkv, Sk, Dh = 32, 32, 32768, 192
        assert Hq % Hkv == 0, (Hq, Hkv)
        return {
            "x": _w((lambda *s: _rng.normal(s) * 0.05)(B, Sq, D)),
            "k_cache": _w((lambda *s: _rng.normal(s) * 0.05)(B, Hkv, Sk, Dh)),
            "v_cache": _w((lambda *s: _rng.normal(s) * 0.05)(B, Hkv, Sk, Dh)),
            "wq": _w((lambda *s: _rng.normal(s) * 0.05)(D, Hq * Dh) * (D ** -0.5)),
            "wo": _w((lambda *s: _rng.normal(s) * 0.05)(Hq * Dh, D) * ((Hq * Dh) ** -0.5)),
        }
    _A_in = _A_setup()

    def _B_setup():
        B, S, D, F = 1, 1, 640, 1536
        return {
            "x": _w((lambda *s: _rng.normal(s) * 0.05)(B, S, D)),
            "w1": _w((lambda *s: _rng.normal(s) * 0.05)(D, F) * (2.0 / D) ** 0.5),
            "w3": _w((lambda *s: _rng.normal(s) * 0.05)(D, F) * (2.0 / D) ** 0.5),
            "w2": _w((lambda *s: _rng.normal(s) * 0.05)(F, D) * (2.0 / F) ** 0.5),
        }
    _B_in = _B_setup()

    return {
        "A_x": _A_in["x"],
        "A_k_cache": _A_in["k_cache"],
        "A_v_cache": _A_in["v_cache"],
        "A_wq": _A_in["wq"],
        "A_wo": _A_in["wo"],
        "B_x": _B_in["x"],
        "B_w1": _B_in["w1"],
        "B_w3": _B_in["w3"],
        "B_w2": _B_in["w2"],
    }

def reference(A_x, A_k_cache, A_v_cache, A_wq, A_wo, B_x, B_w1, B_w3, B_w2):
    def _A_ref(x, k_cache, v_cache, wq, wo):
        B, Sq, D = x.shape
        Hq, Dh = 32, 192
        Hkv, Sk = k_cache.shape[1], k_cache.shape[2]
        W = min(4096, max(256, Sk // 4))
        rep = Hq // Hkv
        q = (lambda x, *d: x.transpose(*d))((x @ wq).reshape(B, Sq, Hq, Dh), 0, 2, 1, 3)
        k = jnp.repeat(k_cache[:, :, Sk - W:, :], rep, axis=1)
        v = jnp.repeat(v_cache[:, :, Sk - W:, :], rep, axis=1)
        scores = jnp.einsum("bhqd,bhkd->bhqk", q, k) * (Dh ** -0.5)
        p = _softmax(scores, axis=-1)
        o = jnp.einsum("bhqk,bhkd->bhqd", p, v)
        return (lambda x, *d: x.transpose(*d))(o, 0, 2, 1, 3).reshape(B, Sq, Hq * Dh) @ wo

    def _B_ref(x, w1, w3, w2):
        gate = jnp.einsum("bsd,df->bsf", x, w1)
        up = jnp.einsum("bsd,df->bsf", x, w3)
        h = _silu(gate) * up
        out = jnp.einsum("bsf,fd->bsd", h, w2)
        return out

    x = A_x
    h = x + _A_ref(_layernorm(x, axis=-1), A_k_cache, A_v_cache, A_wq, A_wo)
    h2 = h + _B_ref(_layernorm(h, axis=-1), B_w1, B_w3, B_w2)
    return h2
```

```python
import functools
import jax
import jax.numpy as jnp
from jax import lax
import jax.experimental.pallas as pl
import jax.experimental.pallas.tpu as pltpu

D = 640
F = 1536
H = 32
DH = 192
G = 2
GD = G * DH
NG = H // G
EPS = 1e-5
NSLOT = 3
WQ_CH = 5
F32 = jnp.float32
BF16 = jnp.bfloat16


def _ln(x):
    m = jnp.mean(x, axis=-1, keepdims=True)
    xc = x - m
    v = jnp.mean(xc * xc, axis=-1, keepdims=True)
    return xc * lax.rsqrt(v + EPS)


def make_kernel(SK, W):
    def kernel(x_hbm, k_hbm, v_hbm, wq_hbm, wo_hbm, w1_hbm, w3_hbm, w2_hbm, o_ref,
               xbuf, wqbuf, kbuf, vbuf, wobuf, w1buf, w3buf, w2buf, q_scr,
               sx, sq, sk, sv, so, s1, s3, s2):
        RQ = D // WQ_CH

        def cx():
            return pltpu.make_async_copy(x_hbm, xbuf, sx)

        def cq(c):
            return pltpu.make_async_copy(wq_hbm.at[pl.ds(c * RQ, RQ), :], wqbuf.at[pl.ds(c * RQ, RQ), :], sq.at[c])

        def ck(j, slot):
            return pltpu.make_async_copy(k_hbm.at[j, :, pl.ds(SK - W, W)], kbuf.at[slot], sk.at[slot])

        def cv(j, slot):
            return pltpu.make_async_copy(v_hbm.at[j, :, pl.ds(SK - W, W)], vbuf.at[slot], sv.at[slot])

        def co(j, slot):
            return pltpu.make_async_copy(wo_hbm.at[pl.ds(pl.multiple_of(j * GD, GD), GD), :], wobuf.at[slot], so.at[slot])

        NF = 5
        RF = D // NF

        def c1(c):
            return pltpu.make_async_copy(w1_hbm.at[pl.ds(c * RF, RF), :], w1buf.at[pl.ds(c * RF, RF), :], s1.at[c])

        def c3(c):
            return pltpu.make_async_copy(w3_hbm.at[pl.ds(c * RF, RF), :], w3buf.at[pl.ds(c * RF, RF), :], s3.at[c])

        N2 = 4
        R2 = F // N2

        def c2(c):
            return pltpu.make_async_copy(w2_hbm.at[pl.ds(c * R2, R2), :], w2buf.at[pl.ds(c * R2, R2), :], s2.at[c])

        cq(0).start()
        cx().start()
        cq(1).start()
        cq(2).start()
        cx().wait()
        x = xbuf[...].astype(F32)
        x8 = jnp.broadcast_to(x, (8, D))
        xn = _ln(x8).astype(BF16)
        q = jnp.zeros((8, H * DH), F32)
        for c in range(WQ_CH):
            cq(c).wait()
            if c + 3 < WQ_CH:
                cq(c + 3).start()
            elif c + 3 == WQ_CH:
                ck(0, 0).start()
            elif c + 3 == WQ_CH + 1:
                cv(0, 0).start()
            elif c + 3 == WQ_CH + 2:
                co(0, 0).start()
                ck(1, 1).start()
            q = q + jnp.dot(xn[:, c * RQ:(c + 1) * RQ], wqbuf[c * RQ:(c + 1) * RQ, :], preferred_element_type=F32)
        q_scr[...] = q.astype(BF16).astype(F32)

        row = lax.broadcasted_iota(jnp.int32, (8, GD), 0)
        col = lax.broadcasted_iota(jnp.int32, (8, GD), 1)
        diag = (col >= row * DH) & (col < (row + 1) * DH)
        scale = DH ** -0.5

        def body(j, acc):
            slot = j % NSLOT
            nslot = (j + 1) % NSLOT
            n2slot = (j + 2) % NSLOT
            ck(j, slot).wait()

            @pl.when(j + 1 < NG)
            def _():
                cv(j + 1, nslot).start()
                co(j + 1, nslot).start()

            @pl.when(j + 1 == NG)
            def _():
                for c in range(NF):
                    c1(c).start()

            qj = q_scr[:, pl.ds(pl.multiple_of(j * GD, 128), GD)]
            qd = jnp.where(diag, qj, 0.0).astype(BF16)
            s = jnp.dot(qd, kbuf[slot], preferred_element_type=F32) * scale
            m = jnp.max(s, axis=-1, keepdims=True)
            p = jnp.exp(s - m)
            l = jnp.sum(p, axis=-1, keepdims=True)
            cv(j, slot).wait()

            @pl.when(j + 2 < NG)
            def _():
                ck(j + 2, n2slot).start()

            @pl.when(j + 1 == NG)
            def _():
                for c in range(NF):
                    c3(c).start()

            o = lax.dot_general(p.astype(BF16), vbuf[slot], (((1,), (1,)), ((), ())), preferred_element_type=F32)
            o = jnp.where(diag, o / l, 0.0).astype(BF16)
            co(j, slot).wait()
            acc = acc + jnp.dot(o, wobuf[slot], preferred_element_type=F32)
            return acc

        acc = lax.fori_loop(0, NG, body, jnp.zeros((8, D), F32))
        attn = jnp.sum(acc, axis=0, keepdims=True)
        h = x + attn
        h8 = jnp.broadcast_to(h, (8, D))
        hn = _ln(h8).astype(BF16)
        for c in range(N2):
            c2(c).start()
        gate = jnp.zeros((8, F), F32)
        up = jnp.zeros((8, F), F32)
        for c in range(NF):
            c1(c).wait()
            gate = gate + jnp.dot(hn[:, c * RF:(c + 1) * RF], w1buf[c * RF:(c + 1) * RF, :], preferred_element_type=F32)
        for c in range(NF):
            c3(c).wait()
            up = up + jnp.dot(hn[:, c * RF:(c + 1) * RF], w3buf[c * RF:(c + 1) * RF, :], preferred_element_type=F32)
        act = (gate * jax.nn.sigmoid(gate) * up).astype(BF16)
        out = h8
        for c in range(N2):
            c2(c).wait()
            out = out + jnp.dot(act[:, c * R2:(c + 1) * R2], w2buf[c * R2:(c + 1) * R2, :], preferred_element_type=F32)
        o_ref[...] = out[0:1, :].astype(o_ref.dtype)
    return kernel


@jax.jit
def pallas_sequential_preLN__sliding_block_cached__glu_gated_swiglu__decode_kernel(
    A_x, A_k_cache, A_v_cache, A_wq, A_wo, B_x, B_w1, B_w3, B_w2
):
    B, Sq, _ = A_x.shape
    _, Hkv, SK, _ = A_k_cache.shape
    W = min(4096, max(256, SK // 4))
    kT = A_k_cache.reshape(H, SK, DH).transpose(0, 2, 1).reshape(NG, GD, SK)
    vT = A_v_cache.reshape(H, SK, DH).transpose(0, 2, 1).reshape(NG, GD, SK)
    x = A_x.reshape(1, D)
    dma = pltpu.SemaphoreType.DMA
    out = pl.pallas_call(
        make_kernel(SK, W),
        out_shape=jax.ShapeDtypeStruct((1, D), A_x.dtype),
        in_specs=[pl.BlockSpec(memory_space=pl.ANY)] * 8,
        out_specs=pl.BlockSpec((1, D), lambda: (0, 0)),
        scratch_shapes=[
            pltpu.VMEM((1, D), BF16),
            pltpu.VMEM((D, H * DH), BF16),
            pltpu.VMEM((NSLOT, GD, W), BF16),
            pltpu.VMEM((NSLOT, GD, W), BF16),
            pltpu.VMEM((NSLOT, GD, D), BF16),
            pltpu.VMEM((D, F), BF16),
            pltpu.VMEM((D, F), BF16),
            pltpu.VMEM((F, D), BF16),
            pltpu.VMEM((8, H * DH), F32),
            dma(()), dma((WQ_CH,)), dma((NSLOT,)), dma((NSLOT,)), dma((NSLOT,)), dma((5,)), dma((5,)), dma((4,)),
        ],
        compiler_params=pltpu.CompilerParams(vmem_limit_bytes=100 * 1024 * 1024),
        name="fused_v1",
    )(x, kT, vT, A_wq, A_wo, B_w1, B_w3, B_w2)
    return out.reshape(B, Sq, D)
```

```python
import functools
import jax
import jax.numpy as jnp
from jax import lax
import jax.experimental.pallas as pl
import jax.experimental.pallas.tpu as pltpu

D = 640
F = 1536
H = 32
DH = 192
EPS = 1e-5
F32 = jnp.float32
BF16 = jnp.bfloat16


def _ln(x):
    m = jnp.mean(x, axis=-1, keepdims=True)
    xc = x - m
    v = jnp.mean(xc * xc, axis=-1, keepdims=True)
    return xc * lax.rsqrt(v + EPS)


def build(name="fused_v4", G=2, dist=1, NSLOT=None, kv_t=(8, 2048), wq_t=(8, 2048), wo_t=(16, 640),
          w13_t=(8, 1536), w2_t=(16, 640), w2_rows=(512, 512, 384, 128), ffn_blk=384, loop_issue=False,
          pat=(0, 1), flags=None):
    GD = G * DH
    NG = H // G
    NSLOT = NSLOT or dist + 1
    N2 = len(w2_rows)
    assert sum(w2_rows) == F
    w2_off = [sum(w2_rows[:i]) for i in range(N2)]

    def make_kernel(SK, W):
        def kernel(x_hbm, k_hbm, v_hbm, wq_hbm, wo_hbm, w1_hbm, w3_hbm, w2_hbm, o_ref,
                   xbuf, wqbuf, kbuf, vbuf, wobuf, w1buf, w3buf, w2buf, act_scr,
                   sx, sq, sk, sv, so, s1, s3, s2):

            def start_tiles(src, dst, sem, nrows, ncols, tile, col0=0):
                tr, tc = tile
                ncol_t = ncols // tc
                nrow_t = nrows // tr
                if not loop_issue:
                    n = 0
                    for i in range(nrow_t):
                        for l in range(ncol_t):
                            pltpu.make_async_copy(
                                src.at[pl.ds(i * tr, tr), pl.ds(col0 + l * tc, tc)],
                                dst.at[pl.ds(i * tr, tr), pl.ds(l * tc, tc)], sem).start(priority=pat[n % len(pat)])
                            n += 1
                else:
                    per = 1 if (ncol_t % len(pat) == 0) else len(pat)
                    assert nrow_t % per == 0

                    def body(i, c):
                        n = 0
                        for u in range(per):
                            r0 = pl.multiple_of((i * per + u) * tr, tr)
                            for l in range(ncol_t):
                                pltpu.make_async_copy(
                                    src.at[pl.ds(r0, tr), pl.ds(col0 + l * tc, tc)],
                                    dst.at[pl.ds(r0, tr), pl.ds(l * tc, tc)], sem).start(priority=pat[n % len(pat)])
                                n += 1
                        return c
                    lax.fori_loop(0, nrow_t // per, body, 0)

            def wait_all(dst, sem):
                pltpu.make_async_copy(dst, dst, sem).wait()

            def start_k(j, slot):
                start_tiles(k_hbm.at[j], kbuf.at[slot], sk.at[slot], GD, W, kv_t, SK - W)

            def start_v(j, slot):
                start_tiles(v_hbm.at[j], vbuf.at[slot], sv.at[slot], GD, W, kv_t, SK - W)

            def start_w1():
                start_tiles(w1_hbm, w1buf, s1, D, F, w13_t)

            def start_w3():
                start_tiles(w3_hbm, w3buf, s3, D, F, w13_t)

            def start_w2():
                for c in range(N2):
                    start_tiles(w2_hbm.at[pl.ds(w2_off[c], w2_rows[c]), :], w2buf.at[pl.ds(w2_off[c], w2_rows[c]), :],
                                s2.at[c], w2_rows[c], D, w2_t)

            pltpu.make_async_copy(x_hbm, xbuf, sx).start()
            start_tiles(wq_hbm, wqbuf, sq, D, H * DH, wq_t)
            start_tiles(wo_hbm, wobuf, so, H * DH, D, wo_t)
            for i in range(2 * dist + 1):
                j = i // 2
                if i % 2 == 0:
                    start_k(j, j % NSLOT)
                else:
                    start_v(j, j % NSLOT)
            pltpu.make_async_copy(x_hbm, xbuf, sx).wait()
            x = xbuf[...].astype(F32)
            x8 = jnp.broadcast_to(x, (8, D))
            xn = _ln(x8).astype(BF16)
            wait_all(wqbuf, sq)
            wait_all(wobuf, so)

            row = lax.broadcasted_iota(jnp.int32, (8, GD), 0)
            col = lax.broadcasted_iota(jnp.int32, (8, GD), 1)
            diag = (col >= row * DH) & (col < (row + 1) * DH)
            scale = DH ** -0.5

            def body(j, acc):
                slot = lax.rem(j, NSLOT)
                nslot = lax.rem(j + dist, NSLOT)
                n2slot = lax.rem(j + dist + 1, NSLOT)
                off = pl.multiple_of(j * GD, 128)
                q = jnp.dot(xn, wqbuf[:, pl.ds(off, GD)], preferred_element_type=F32)
                qd = jnp.where(diag, q, 0.0).astype(BF16)
                wait_all(kbuf.at[slot], sk.at[slot])

                @pl.when(j + dist < NG)
                def _():
                    start_v(j + dist, nslot)

                @pl.when(j + dist == NG)
                def _():
                    start_w1()

                s = jnp.dot(qd, kbuf[slot], preferred_element_type=F32) * scale
                m = jnp.max(s, axis=-1, keepdims=True)
                p = jnp.exp(s - m)
                l = jnp.sum(p, axis=-1, keepdims=True)
                wait_all(vbuf.at[slot], sv.at[slot])

                @pl.when(j + dist + 1 < NG)
                def _():
                    start_k(j + dist + 1, n2slot)

                @pl.when(j + dist == NG)
                def _():
                    start_w3()

                o = lax.dot_general(p.astype(BF16), vbuf[slot], (((1,), (1,)), ((), ())), preferred_element_type=F32)
                o = jnp.where(diag, o / l, 0.0).astype(BF16)
                acc = acc + jnp.dot(o, wobuf[pl.ds(off, GD), :], preferred_element_type=F32)
                return acc

            acc = lax.fori_loop(0, NG, body, jnp.zeros((8, D), F32))
            start_w2()
            attn = jnp.sum(acc, axis=0, keepdims=True)
            h = x + attn
            h8 = jnp.broadcast_to(h, (8, D))
            hn = _ln(h8).astype(BF16)

            wait_all(w1buf, s1)

            def gate_body(b, carry):
                off = pl.multiple_of(b * ffn_blk, 128)
                act_scr[:, pl.ds(off, ffn_blk)] = jnp.dot(hn, w1buf[:, pl.ds(off, ffn_blk)], preferred_element_type=F32)
                return carry
            lax.fori_loop(0, F // ffn_blk, gate_body, 0)

            wait_all(w3buf, s3)

            def up_body(b, carry):
                off = pl.multiple_of(b * ffn_blk, 128)
                up = jnp.dot(hn, w3buf[:, pl.ds(off, ffn_blk)], preferred_element_type=F32)
                g = act_scr[:, pl.ds(off, ffn_blk)]
                act_scr[:, pl.ds(off, ffn_blk)] = g * jax.nn.sigmoid(g) * up
                return carry
            lax.fori_loop(0, F // ffn_blk, up_body, 0)

            out = h8
            for c in range(N2):
                a = act_scr[:, w2_off[c]:w2_off[c] + w2_rows[c]].astype(BF16)
                wait_all(w2buf.at[pl.ds(w2_off[c], w2_rows[c]), :], s2.at[c])
                out = out + jnp.dot(a, w2buf[w2_off[c]:w2_off[c] + w2_rows[c], :], preferred_element_type=F32)
            o_ref[...] = out[0:1, :].astype(o_ref.dtype)
        return kernel

    @jax.jit
    def kernel_fn(A_x, A_k_cache, A_v_cache, A_wq, A_wo, B_x, B_w1, B_w3, B_w2):
        B, Sq, _ = A_x.shape
        _, Hkv, SK, _ = A_k_cache.shape
        W = min(4096, max(256, SK // 4))
        kT = A_k_cache.reshape(H, SK, DH).transpose(0, 2, 1).reshape(NG, GD, SK)
        vT = A_v_cache.reshape(H, SK, DH).transpose(0, 2, 1).reshape(NG, GD, SK)
        x = A_x.reshape(1, D)
        dma = pltpu.SemaphoreType.DMA
        out = pl.pallas_call(
            make_kernel(SK, W),
            out_shape=jax.ShapeDtypeStruct((1, D), A_x.dtype),
            in_specs=[pl.BlockSpec(memory_space=pl.ANY)] * 8,
            out_specs=pl.BlockSpec((1, D), lambda: (0, 0)),
            scratch_shapes=[
                pltpu.VMEM((1, D), BF16),
                pltpu.VMEM((D, H * DH), BF16),
                pltpu.VMEM((NSLOT, GD, W), BF16),
                pltpu.VMEM((NSLOT, GD, W), BF16),
                pltpu.VMEM((H * DH, D), BF16),
                pltpu.VMEM((D, F), BF16),
                pltpu.VMEM((D, F), BF16),
                pltpu.VMEM((F, D), BF16),
                pltpu.VMEM((8, F), F32),
                dma(()), dma(()), dma((NSLOT,)), dma((NSLOT,)), dma(()), dma(()), dma(()), dma((N2,)),
            ],
            compiler_params=pltpu.CompilerParams(vmem_limit_bytes=110 * 1024 * 1024, disable_bounds_checks=True,
                                                 disable_semaphore_checks=True, flags=flags),
            name=name,
        )(x, kT, vT, A_wq, A_wo, B_w1, B_w3, B_w2)
        return out.reshape(B, Sq, D)
    return kernel_fn


_kernel_fn = build(name="fused_v4", loop_issue=True)


def pallas_sequential_preLN__sliding_block_cached__glu_gated_swiglu__decode_kernel(
    A_x, A_k_cache, A_v_cache, A_wq, A_wo, B_x, B_w1, B_w3, B_w2
):
    return _kernel_fn(A_x, A_k_cache, A_v_cache, A_wq, A_wo, B_x, B_w1, B_w3, B_w2)
```

```python
import functools
import jax
import jax.numpy as jnp
from jax import lax
import jax.experimental.pallas as pl
import jax.experimental.pallas.tpu as pltpu

D = 640
F = 1536
H = 32
DH = 192
EPS = 1e-5
F32 = jnp.float32
BF16 = jnp.bfloat16


def _ln(x):
    m = jnp.mean(x, axis=-1, keepdims=True)
    xc = x - m
    v = jnp.mean(xc * xc, axis=-1, keepdims=True)
    return xc * lax.rsqrt(v + EPS)


def build(name="fused_v6", G=2, dist=1, NSLOT=None, kv_t=(8, 2048, 'half'), wq_t=(8, 2048), wo_t=(16, 640),
          w13_t=(8, 1536), w2_t=(16, 640), w2_rows=(512, 512, 384, 128), ffn_blk=384, loop_issue=True,
          pat=(0, 1), flags=None, compute_first=False, w2_split=0):
    GD = G * DH
    NG = H // G
    NSLOT = NSLOT or dist + 1
    N2 = len(w2_rows)
    assert sum(w2_rows) == F
    w2_off = [sum(w2_rows[:i]) for i in range(N2)]

    def make_kernel(SK, W):
        def kernel(x_hbm, k_hbm, v_hbm, wq_hbm, wo_hbm, w1_hbm, w3_hbm, w2_hbm, o_ref,
                   xbuf, wqbuf, kbuf, vbuf, wobuf, w1buf, w3buf, w2buf, act_scr,
                   sx, sq, sk, sv, so, s1, s3, s2):

            def start_tiles(src, dst, sem, nrows, ncols, tile, col0=0):
                tr, tc = tile[0], tile[1]
                mode = tile[2] if len(tile) > 2 else 'rm'
                ncol_t = ncols // tc
                nrow_t = nrows // tr
                def cp(r, l, pr):
                    r0 = pl.multiple_of(r * tr, tr)
                    pltpu.make_async_copy(src.at[pl.ds(r0, tr), pl.ds(col0 + l * tc, tc)],
                                          dst.at[pl.ds(r0, tr), pl.ds(l * tc, tc)], sem).start(priority=pr)
                if mode == 'rm':
                    per = 1 if (ncol_t % 2 == 0) else 2
                    def body(i, c):
                        n = 0
                        for u in range(per):
                            for l in range(ncol_t):
                                cp(i * per + u, l, n % 2); n += 1
                        return c
                    lax.fori_loop(0, nrow_t // per, body, 0)
                elif mode == 'cm':
                    for l in range(ncol_t):
                        def body(i, c):
                            cp(2 * i, l, 0); cp(2 * i + 1, l, 1)
                            return c
                        lax.fori_loop(0, nrow_t // 2, body, 0)
                elif mode == 'half':
                    def body(i, c):
                        for l in range(ncol_t):
                            cp(i, l, 0); cp(i + nrow_t // 2, l, 1)
                        return c
                    lax.fori_loop(0, nrow_t // 2, body, 0)
                elif mode == 'halfcm':
                    for l in range(ncol_t):
                        def body(i, c):
                            cp(i, l, 0); cp(i + nrow_t // 2, l, 1)
                            return c
                        lax.fori_loop(0, nrow_t // 2, body, 0)
                elif mode[0] == 's':
                    A = int(mode[1:]); B = nrow_t // A
                    assert A * B == nrow_t and A % 2 == 0
                    def body(bi, c):
                        n = 0
                        for a in range(A):
                            for l in range(ncol_t):
                                cp(a * B + bi, l, n % 2); n += 1
                        return c
                    lax.fori_loop(0, B, body, 0)
                else:
                    raise ValueError(mode)

            def wait_all(dst, sem):
                pltpu.make_async_copy(dst, dst, sem).wait()

            def start_k(j, slot):
                start_tiles(k_hbm.at[j], kbuf.at[slot], sk.at[slot], GD, W, kv_t, SK - W)

            def start_v(j, slot):
                start_tiles(v_hbm.at[j], vbuf.at[slot], sv.at[slot], GD, W, kv_t, SK - W)

            def start_w1():
                start_tiles(w1_hbm, w1buf, s1, D, F, w13_t)

            def start_w3():
                start_tiles(w3_hbm, w3buf, s3, D, F, w13_t)

            def w2tile(c):
                t = w2_t[c] if isinstance(w2_t, list) else w2_t
                return t

            def start_w2(chunks):
                for c in chunks:
                    start_tiles(w2_hbm.at[pl.ds(w2_off[c], w2_rows[c]), :], w2buf.at[pl.ds(w2_off[c], w2_rows[c]), :],
                                s2.at[c], w2_rows[c], D, w2tile(c))

            pltpu.make_async_copy(x_hbm, xbuf, sx).start()
            start_tiles(wq_hbm, wqbuf, sq, D, H * DH, wq_t)
            start_tiles(wo_hbm, wobuf, so, H * DH, D, wo_t)
            for i in range(2 * dist + 1):
                j = i // 2
                if i % 2 == 0:
                    start_k(j, j % NSLOT)
                else:
                    start_v(j, j % NSLOT)
            pltpu.make_async_copy(x_hbm, xbuf, sx).wait()
            x = xbuf[...].astype(F32)
            x8 = jnp.broadcast_to(x, (8, D))
            xn = _ln(x8).astype(BF16)
            wait_all(wqbuf, sq)
            wait_all(wobuf, so)

            row = lax.broadcasted_iota(jnp.int32, (8, GD), 0)
            col = lax.broadcasted_iota(jnp.int32, (8, GD), 1)
            diag = (col >= row * DH) & (col < (row + 1) * DH)
            scale = DH ** -0.5

            def body(j, acc):
                slot = lax.rem(j, NSLOT)
                nslot = lax.rem(j + dist, NSLOT)
                n2slot = lax.rem(j + dist + 1, NSLOT)
                off = pl.multiple_of(j * GD, 128)

                def issue_a():
                    @pl.when(j + dist < NG)
                    def _():
                        start_v(j + dist, nslot)

                    @pl.when(j + dist == NG)
                    def _():
                        start_w1()

                def issue_b():
                    @pl.when(j + dist + 1 < NG)
                    def _():
                        start_k(j + dist + 1, n2slot)

                    @pl.when(j + dist == NG)
                    def _():
                        start_w3()

                q = jnp.dot(xn, wqbuf[:, pl.ds(off, GD)], preferred_element_type=F32)
                qd = jnp.where(diag, q, 0.0).astype(BF16)
                wait_all(kbuf.at[slot], sk.at[slot])
                if not compute_first:
                    issue_a()
                s = jnp.dot(qd, kbuf[slot], preferred_element_type=F32) * scale
                m = jnp.max(s, axis=-1, keepdims=True)
                p = jnp.exp(s - m)
                l = jnp.sum(p, axis=-1, keepdims=True)
                if compute_first:
                    issue_a()
                wait_all(vbuf.at[slot], sv.at[slot])
                if not compute_first:
                    issue_b()
                o = lax.dot_general(p.astype(BF16), vbuf[slot], (((1,), (1,)), ((), ())), preferred_element_type=F32)
                o = jnp.where(diag, o / l, 0.0).astype(BF16)
                acc = acc + jnp.dot(o, wobuf[pl.ds(off, GD), :], preferred_element_type=F32)
                if compute_first:
                    issue_b()
                return acc

            acc = lax.fori_loop(0, NG, body, jnp.zeros((8, D), F32))
            if w2_split == 0:
                start_w2(range(N2))
            attn = jnp.sum(acc, axis=0, keepdims=True)
            h = x + attn
            h8 = jnp.broadcast_to(h, (8, D))
            hn = _ln(h8).astype(BF16)

            wait_all(w1buf, s1)

            def gate_body(b, carry):
                off = pl.multiple_of(b * ffn_blk, 128)
                act_scr[:, pl.ds(off, ffn_blk)] = jnp.dot(hn, w1buf[:, pl.ds(off, ffn_blk)], preferred_element_type=F32)
                return carry
            lax.fori_loop(0, F // ffn_blk, gate_body, 0)

            if w2_split > 0:
                start_w2(range(w2_split))
            wait_all(w3buf, s3)

            def up_body(b, carry):
                off = pl.multiple_of(b * ffn_blk, 128)
                up = jnp.dot(hn, w3buf[:, pl.ds(off, ffn_blk)], preferred_element_type=F32)
                g = act_scr[:, pl.ds(off, ffn_blk)]
                act_scr[:, pl.ds(off, ffn_blk)] = g * jax.nn.sigmoid(g) * up
                return carry
            lax.fori_loop(0, F // ffn_blk, up_body, 0)

            if w2_split > 0:
                start_w2(range(w2_split, N2))
            out = h8
            for c in range(N2):
                a = act_scr[:, w2_off[c]:w2_off[c] + w2_rows[c]].astype(BF16)
                wait_all(w2buf.at[pl.ds(w2_off[c], w2_rows[c]), :], s2.at[c])
                out = out + jnp.dot(a, w2buf[w2_off[c]:w2_off[c] + w2_rows[c], :], preferred_element_type=F32)
            o_ref[...] = out[0:1, :].astype(o_ref.dtype)
        return kernel

    @jax.jit
    def kernel_fn(A_x, A_k_cache, A_v_cache, A_wq, A_wo, B_x, B_w1, B_w3, B_w2):
        B, Sq, _ = A_x.shape
        _, Hkv, SK, _ = A_k_cache.shape
        W = min(4096, max(256, SK // 4))
        kT = A_k_cache.reshape(H, SK, DH).transpose(0, 2, 1).reshape(NG, GD, SK)
        vT = A_v_cache.reshape(H, SK, DH).transpose(0, 2, 1).reshape(NG, GD, SK)
        x = A_x.reshape(1, D)
        dma = pltpu.SemaphoreType.DMA
        out = pl.pallas_call(
            make_kernel(SK, W),
            out_shape=jax.ShapeDtypeStruct((1, D), A_x.dtype),
            in_specs=[pl.BlockSpec(memory_space=pl.ANY)] * 8,
            out_specs=pl.BlockSpec((1, D), lambda: (0, 0)),
            scratch_shapes=[
                pltpu.VMEM((1, D), BF16),
                pltpu.VMEM((D, H * DH), BF16),
                pltpu.VMEM((NSLOT, GD, W), BF16),
                pltpu.VMEM((NSLOT, GD, W), BF16),
                pltpu.VMEM((H * DH, D), BF16),
                pltpu.VMEM((D, F), BF16),
                pltpu.VMEM((D, F), BF16),
                pltpu.VMEM((F, D), BF16),
                pltpu.VMEM((8, F), F32),
                dma(()), dma(()), dma((NSLOT,)), dma((NSLOT,)), dma(()), dma(()), dma(()), dma((N2,)),
            ],
            compiler_params=pltpu.CompilerParams(vmem_limit_bytes=110 * 1024 * 1024, disable_bounds_checks=True,
                                                 disable_semaphore_checks=True, flags=flags),
            name=name,
        )(x, kT, vT, A_wq, A_wo, B_w1, B_w3, B_w2)
        return out.reshape(B, Sq, D)
    return kernel_fn


_kernel_fn = build(name="fused_decode", wq_t=(8, 2048, 's8'), wo_t=(16, 640, 's8'), w13_t=(8, 1536, 's8'), w2_t=(16, 640, 's8'))


def pallas_sequential_preLN__sliding_block_cached__glu_gated_swiglu__decode_kernel(
    A_x, A_k_cache, A_v_cache, A_wq, A_wo, B_x, B_w1, B_w3, B_w2
):
    return _kernel_fn(A_x, A_k_cache, A_v_cache, A_wq, A_wo, B_x, B_w1, B_w3, B_w2)
```

```python
import functools
import jax
import jax.numpy as jnp
from jax import lax
import jax.experimental.pallas as pl
import jax.experimental.pallas.tpu as pltpu

D = 640
F = 1536
H = 32
DH = 192
EPS = 1e-5
F32 = jnp.float32
BF16 = jnp.bfloat16


def _ln(x):
    m = jnp.mean(x, axis=-1, keepdims=True)
    xc = x - m
    v = jnp.mean(xc * xc, axis=-1, keepdims=True)
    return xc * lax.rsqrt(v + EPS)


def build(name="fused_v6", G=2, dist=1, NSLOT=None, kv_t=(8, 2048, 'half'), wq_t=(8, 2048), wo_t=(16, 640),
          w13_t=(8, 1536), w2_t=(16, 640), w2_rows=(512, 512, 384, 128), ffn_blk=384, loop_issue=True,
          pat=(0, 1), flags=None, compute_first=False, w2_split=0):
    GD = G * DH
    NG = H // G
    NSLOT = NSLOT or dist + 1
    N2 = len(w2_rows)
    assert sum(w2_rows) == F
    w2_off = [sum(w2_rows[:i]) for i in range(N2)]

    def make_kernel(SK, W):
        def kernel(x_hbm, k_hbm, v_hbm, wq_hbm, wo_hbm, w1_hbm, w3_hbm, w2_hbm, o_ref,
                   xbuf, wqbuf, kbuf, vbuf, wobuf, w1buf, w3buf, w2buf, act_scr,
                   sx, sq, sk, sv, so, s1, s3, s2):

            def start_tiles(src, dst, sem, nrows, ncols, tile, col0=0):
                tr, tc = tile[0], tile[1]
                mode = tile[2] if len(tile) > 2 else 'rm'
                ncol_t = ncols // tc
                nrow_t = nrows // tr
                def cp(r, l, pr):
                    r0 = pl.multiple_of(r * tr, tr)
                    pltpu.make_async_copy(src.at[pl.ds(r0, tr), pl.ds(col0 + l * tc, tc)],
                                          dst.at[pl.ds(r0, tr), pl.ds(l * tc, tc)], sem).start(priority=pr)
                if mode == 'rm':
                    per = 1 if (ncol_t % 2 == 0) else 2
                    def body(i, c):
                        n = 0
                        for u in range(per):
                            for l in range(ncol_t):
                                cp(i * per + u, l, n % 2); n += 1
                        return c
                    lax.fori_loop(0, nrow_t // per, body, 0)
                elif mode == 'cm':
                    for l in range(ncol_t):
                        def body(i, c):
                            cp(2 * i, l, 0); cp(2 * i + 1, l, 1)
                            return c
                        lax.fori_loop(0, nrow_t // 2, body, 0)
                elif mode == 'half':
                    def body(i, c):
                        for l in range(ncol_t):
                            cp(i, l, 0); cp(i + nrow_t // 2, l, 1)
                        return c
                    lax.fori_loop(0, nrow_t // 2, body, 0)
                elif mode == 'halfcm':
                    for l in range(ncol_t):
                        def body(i, c):
                            cp(i, l, 0); cp(i + nrow_t // 2, l, 1)
                            return c
                        lax.fori_loop(0, nrow_t // 2, body, 0)
                elif mode == 'pair':
                    def body(i, c):
                        for l in range(ncol_t):
                            cp(2 * i, l, 0); cp(2 * i + 1, l, 1)
                        return c
                    lax.fori_loop(0, nrow_t // 2, body, 0)
                elif mode == 'rm10':
                    per = 1 if (ncol_t % 2 == 0) else 2
                    def body(i, c):
                        n = 1
                        for u in range(per):
                            for l in range(ncol_t):
                                cp(i * per + u, l, n % 2); n += 1
                        return c
                    lax.fori_loop(0, nrow_t // per, body, 0)
                elif mode == 'zig':
                    def body(i, c):
                        for u in range(2):
                            for l in range(ncol_t):
                                cp(2 * i + u, l, (l + u) % 2)
                        return c
                    lax.fori_loop(0, nrow_t // 2, body, 0)
                elif mode[0] == 's':
                    A = int(mode[1:]); B = nrow_t // A
                    assert A * B == nrow_t and A % 2 == 0
                    def body(bi, c):
                        n = 0
                        for a in range(A):
                            for l in range(ncol_t):
                                cp(a * B + bi, l, n % 2); n += 1
                        return c
                    lax.fori_loop(0, B, body, 0)
                else:
                    raise ValueError(mode)

            def wait_all(dst, sem):
                pltpu.make_async_copy(dst, dst, sem).wait()

            def start_k(j, slot):
                start_tiles(k_hbm.at[j], kbuf.at[slot], sk.at[slot], GD, W, kv_t, SK - W)

            def start_v(j, slot):
                start_tiles(v_hbm.at[j], vbuf.at[slot], sv.at[slot], GD, W, kv_t, SK - W)

            def start_w1():
                start_tiles(w1_hbm, w1buf, s1, D, F, w13_t)

            def start_w3():
                start_tiles(w3_hbm, w3buf, s3, D, F, w13_t)

            def w2tile(c):
                t = w2_t[c] if isinstance(w2_t, list) else w2_t
                return t

            def start_w2(chunks):
                for c in chunks:
                    start_tiles(w2_hbm.at[pl.ds(w2_off[c], w2_rows[c]), :], w2buf.at[pl.ds(w2_off[c], w2_rows[c]), :],
                                s2.at[c], w2_rows[c], D, w2tile(c))

            pltpu.make_async_copy(x_hbm, xbuf, sx).start()
            start_tiles(wq_hbm, wqbuf, sq, D, H * DH, wq_t)
            start_tiles(wo_hbm, wobuf, so, H * DH, D, wo_t)
            for i in range(2 * dist + 1):
                j = i // 2
                if i % 2 == 0:
                    start_k(j, j % NSLOT)
                else:
                    start_v(j, j % NSLOT)
            pltpu.make_async_copy(x_hbm, xbuf, sx).wait()
            x = xbuf[...].astype(F32)
            x8 = jnp.broadcast_to(x, (8, D))
            xn = _ln(x8).astype(BF16)
            wait_all(wqbuf, sq)
            wait_all(wobuf, so)

            row = lax.broadcasted_iota(jnp.int32, (8, GD), 0)
            col = lax.broadcasted_iota(jnp.int32, (8, GD), 1)
            diag = (col >= row * DH) & (col < (row + 1) * DH)
            scale = DH ** -0.5

            def body(j, acc):
                slot = lax.rem(j, NSLOT)
                nslot = lax.rem(j + dist, NSLOT)
                n2slot = lax.rem(j + dist + 1, NSLOT)
                off = pl.multiple_of(j * GD, 128)

                def issue_a():
                    @pl.when(j + dist < NG)
                    def _():
                        start_v(j + dist, nslot)

                    @pl.when(j + dist == NG)
                    def _():
                        start_w1()

                def issue_b():
                    @pl.when(j + dist + 1 < NG)
                    def _():
                        start_k(j + dist + 1, n2slot)

                    @pl.when(j + dist == NG)
                    def _():
                        start_w3()

                q = jnp.dot(xn, wqbuf[:, pl.ds(off, GD)], preferred_element_type=F32)
                qd = jnp.where(diag, q, 0.0).astype(BF16)
                wait_all(kbuf.at[slot], sk.at[slot])
                if not compute_first:
                    issue_a()
                s = jnp.dot(qd, kbuf[slot], preferred_element_type=F32) * scale
                m = jnp.max(s, axis=-1, keepdims=True)
                p = jnp.exp(s - m)
                l = jnp.sum(p, axis=-1, keepdims=True)
                if compute_first:
                    issue_a()
                wait_all(vbuf.at[slot], sv.at[slot])
                if not compute_first:
                    issue_b()
                o = lax.dot_general(p.astype(BF16), vbuf[slot], (((1,), (1,)), ((), ())), preferred_element_type=F32)
                o = jnp.where(diag, o / l, 0.0).astype(BF16)
                acc = acc + jnp.dot(o, wobuf[pl.ds(off, GD), :], preferred_element_type=F32)
                if compute_first:
                    issue_b()
                return acc

            acc = lax.fori_loop(0, NG, body, jnp.zeros((8, D), F32))
            if w2_split == 0:
                start_w2(range(N2))
            attn = jnp.sum(acc, axis=0, keepdims=True)
            h = x + attn
            h8 = jnp.broadcast_to(h, (8, D))
            hn = _ln(h8).astype(BF16)

            wait_all(w1buf, s1)

            def gate_body(b, carry):
                off = pl.multiple_of(b * ffn_blk, 128)
                act_scr[:, pl.ds(off, ffn_blk)] = jnp.dot(hn, w1buf[:, pl.ds(off, ffn_blk)], preferred_element_type=F32)
                return carry
            lax.fori_loop(0, F // ffn_blk, gate_body, 0)

            if w2_split > 0:
                start_w2(range(w2_split))
            wait_all(w3buf, s3)

            def up_body(b, carry):
                off = pl.multiple_of(b * ffn_blk, 128)
                up = jnp.dot(hn, w3buf[:, pl.ds(off, ffn_blk)], preferred_element_type=F32)
                g = act_scr[:, pl.ds(off, ffn_blk)]
                act_scr[:, pl.ds(off, ffn_blk)] = g * jax.nn.sigmoid(g) * up
                return carry
            lax.fori_loop(0, F // ffn_blk, up_body, 0)

            if w2_split > 0:
                start_w2(range(w2_split, N2))
            out = h8
            for c in range(N2):
                a = act_scr[:, w2_off[c]:w2_off[c] + w2_rows[c]].astype(BF16)
                wait_all(w2buf.at[pl.ds(w2_off[c], w2_rows[c]), :], s2.at[c])
                out = out + jnp.dot(a, w2buf[w2_off[c]:w2_off[c] + w2_rows[c], :], preferred_element_type=F32)
            o_ref[...] = out[0:1, :].astype(o_ref.dtype)
        return kernel

    @jax.jit
    def kernel_fn(A_x, A_k_cache, A_v_cache, A_wq, A_wo, B_x, B_w1, B_w3, B_w2):
        B, Sq, _ = A_x.shape
        _, Hkv, SK, _ = A_k_cache.shape
        W = min(4096, max(256, SK // 4))
        kT = A_k_cache.reshape(H, SK, DH).transpose(0, 2, 1).reshape(NG, GD, SK)
        vT = A_v_cache.reshape(H, SK, DH).transpose(0, 2, 1).reshape(NG, GD, SK)
        x = A_x.reshape(1, D)
        dma = pltpu.SemaphoreType.DMA
        out = pl.pallas_call(
            make_kernel(SK, W),
            out_shape=jax.ShapeDtypeStruct((1, D), A_x.dtype),
            in_specs=[pl.BlockSpec(memory_space=pl.ANY)] * 8,
            out_specs=pl.BlockSpec((1, D), lambda: (0, 0)),
            scratch_shapes=[
                pltpu.VMEM((1, D), BF16),
                pltpu.VMEM((D, H * DH), BF16),
                pltpu.VMEM((NSLOT, GD, W), BF16),
                pltpu.VMEM((NSLOT, GD, W), BF16),
                pltpu.VMEM((H * DH, D), BF16),
                pltpu.VMEM((D, F), BF16),
                pltpu.VMEM((D, F), BF16),
                pltpu.VMEM((F, D), BF16),
                pltpu.VMEM((8, F), F32),
                dma(()), dma(()), dma((NSLOT,)), dma((NSLOT,)), dma(()), dma(()), dma(()), dma((N2,)),
            ],
            compiler_params=pltpu.CompilerParams(vmem_limit_bytes=110 * 1024 * 1024, disable_bounds_checks=True,
                                                 disable_semaphore_checks=True, flags=flags),
            name=name,
        )(x, kT, vT, A_wq, A_wo, B_w1, B_w3, B_w2)
        return out.reshape(B, Sq, D)
    return kernel_fn


_kernel_fn = build(name="fused_decode", kv_t=(8, 2048, 'cm'), wq_t=(8, 2048, 's8'), wo_t=(16, 640, 's8'), w13_t=(8, 1536, 's8'), w2_t=(16, 640, 's8'))


def pallas_sequential_preLN__sliding_block_cached__glu_gated_swiglu__decode_kernel(
    A_x, A_k_cache, A_v_cache, A_wq, A_wo, B_x, B_w1, B_w3, B_w2
):
    return _kernel_fn(A_x, A_k_cache, A_v_cache, A_wq, A_wo, B_x, B_w1, B_w3, B_w2)
```

```python
import jax
import jax.numpy as jnp
from jax import lax
import jax.experimental.pallas as pl
import jax.experimental.pallas.tpu as pltpu

_EPS = 1e-5
_HEAD_DIM = 192
_GROUP = 2
_GD = _GROUP * _HEAD_DIM
_NSLOT = 2
_ROWS = 8
_FFN_BLK = 384
_W2_ROWS = (512, 512, 384, 128)
_STRIPES = 8

_S_PRO, _S_K, _S_V, _S_W13, _NSEM = 0, 1, 3, 5, 6


def _layernorm(x):
    mean = jnp.mean(x, axis=-1, keepdims=True)
    xc = x - mean
    var = jnp.mean(xc * xc, axis=-1, keepdims=True)
    return xc * lax.rsqrt(var + _EPS)


def _start_tile(src, dst, sem, row0, rows, src_col, dst_col, cols, thread):
    pltpu.make_async_copy(
        src.at[pl.ds(row0, rows), pl.ds(src_col, cols)],
        dst.at[pl.ds(row0, rows), pl.ds(dst_col, cols)],
        sem,
    ).start(priority=thread)


def _start_striped(src, dst, sem, tile_rows, tile_cols):
    n_rows, n_cols = dst.shape
    per_stripe = n_rows // (tile_rows * _STRIPES)
    assert per_stripe * tile_rows * _STRIPES == n_rows and n_cols % tile_cols == 0

    def body(i, carry):
        for c in range(0, n_cols, tile_cols):
            for s in range(_STRIPES):
                row0 = pl.multiple_of((s * per_stripe + i) * tile_rows, tile_rows)
                _start_tile(src, dst, sem, row0, tile_rows, c, c, tile_cols, s % 2)
        return carry

    if per_stripe == 1:
        body(0, None)
    else:
        lax.fori_loop(0, per_stripe, body, None)


def _start_window(src, dst, sem, col0):
    n_rows, width = dst.shape
    half = width // 2
    for c in (0, half):
        def body(i, carry, c=c):
            for t in range(2):
                row0 = pl.multiple_of((2 * i + t) * 8, 8)
                _start_tile(src, dst, sem, row0, 8, col0 + c, c, half, t)
            return carry

        lax.fori_loop(0, n_rows // 16, body, None)


def _wait_all(dst, sem):
    pltpu.make_async_copy(dst, dst, sem).wait()


def _kernel(x_hbm, k_hbm, v_hbm, wq_hbm, wo_hbm, w1_hbm, w3_hbm, w2_hbm, o_ref,
            xbuf, wqbuf, wobuf, kbuf, vbuf, w1buf, w3buf, w2buf, act_scr, sems,
            *, window):
    f32, bf16 = jnp.float32, jnp.bfloat16
    n_groups, _, seq = k_hbm.shape
    d_model = xbuf.shape[1]
    d_ffn = w1buf.shape[1]
    col0 = seq - window

    def start_k(j):
        slot = j % _NSLOT
        _start_window(k_hbm.at[j], kbuf.at[slot], sems.at[_S_K + slot], col0)

    def start_v(j):
        slot = j % _NSLOT
        _start_window(v_hbm.at[j], vbuf.at[slot], sems.at[_S_V + slot], col0)

    pro = sems.at[_S_PRO]
    pltpu.make_async_copy(x_hbm, xbuf, pro).start()
    _start_striped(wq_hbm, wqbuf, pro, 8, 2048)
    _start_striped(wo_hbm, wobuf, pro, 16, d_model)
    start_k(0)
    start_v(0)
    start_k(1)
    _wait_all(xbuf, pro)
    _wait_all(wqbuf, pro)
    _wait_all(wobuf, pro)

    x = xbuf[...].astype(f32)
    xn = _layernorm(jnp.broadcast_to(x, (_ROWS, d_model))).astype(bf16)

    row = lax.broadcasted_iota(jnp.int32, (_ROWS, _GD), 0)
    col = lax.broadcasted_iota(jnp.int32, (_ROWS, _GD), 1)
    diag = (col >= row * _HEAD_DIM) & (col < (row + 1) * _HEAD_DIM)
    scale = _HEAD_DIM ** -0.5

    def group(j, acc):
        slot = j % _NSLOT
        off = pl.multiple_of(j * _GD, 128)
        q = jnp.dot(xn, wqbuf[:, pl.ds(off, _GD)], preferred_element_type=f32)
        q = jnp.where(diag, q, 0.0).astype(bf16)

        _wait_all(kbuf.at[slot], sems.at[_S_K + slot])

        @pl.when(j + 1 < n_groups)
        def _():
            start_v(j + 1)

        @pl.when(j + 1 == n_groups)
        def _():
            _start_striped(w1_hbm, w1buf, sems.at[_S_W13], 8, d_ffn)

        s = jnp.dot(q, kbuf[slot], preferred_element_type=f32) * scale
        p = jnp.exp(s - jnp.max(s, axis=-1, keepdims=True))
        l = jnp.sum(p, axis=-1, keepdims=True)

        _wait_all(vbuf.at[slot], sems.at[_S_V + slot])

        @pl.when(j + 2 < n_groups)
        def _():
            start_k(j + 2)

        @pl.when(j + 1 == n_groups)
        def _():
            _start_striped(w3_hbm, w3buf, sems.at[_S_W13], 8, d_ffn)

        o = lax.dot_general(p.astype(bf16), vbuf[slot], (((1,), (1,)), ((), ())),
                            preferred_element_type=f32)
        o = jnp.where(diag, o / l, 0.0).astype(bf16)
        return acc + jnp.dot(o, wobuf[pl.ds(off, _GD), :], preferred_element_type=f32)

    acc = lax.fori_loop(0, n_groups, group, jnp.zeros((_ROWS, d_model), f32))

    w2_chunks = []
    lo = 0
    for c, rows in enumerate(_W2_ROWS):
        sem = sems.at[_S_K + c]
        _start_striped(w2_hbm.at[pl.ds(lo, rows), :], w2buf.at[pl.ds(lo, rows), :],
                       sem, 16, d_model)
        w2_chunks.append((lo, rows, sem))
        lo += rows

    h = x + jnp.sum(acc, axis=0, keepdims=True)
    h = jnp.broadcast_to(h, (_ROWS, d_model))
    hn = _layernorm(h).astype(bf16)

    _wait_all(w1buf, sems.at[_S_W13])
    _wait_all(w3buf, sems.at[_S_W13])

    def ffn_block(b, carry):
        off = pl.multiple_of(b * _FFN_BLK, 128)
        gate = jnp.dot(hn, w1buf[:, pl.ds(off, _FFN_BLK)], preferred_element_type=f32)
        up = jnp.dot(hn, w3buf[:, pl.ds(off, _FFN_BLK)], preferred_element_type=f32)
        act_scr[:, pl.ds(off, _FFN_BLK)] = gate * jax.nn.sigmoid(gate) * up
        return carry

    lax.fori_loop(0, d_ffn // _FFN_BLK, ffn_block, None)

    out = h
    for lo, rows, sem in w2_chunks:
        act = act_scr[:, lo:lo + rows].astype(bf16)
        _wait_all(w2buf.at[pl.ds(lo, rows), :], sem)
        out = out + jnp.dot(act, w2buf[lo:lo + rows, :], preferred_element_type=f32)
    o_ref[...] = out[0:1, :].astype(o_ref.dtype)


def pallas_sequential_preLN__sliding_block_cached__glu_gated_swiglu__decode_kernel(
    A_x: jax.Array,
    A_k_cache: jax.Array,
    A_v_cache: jax.Array,
    A_wq: jax.Array,
    A_wo: jax.Array,
    B_x: jax.Array,
    B_w1: jax.Array,
    B_w3: jax.Array,
    B_w2: jax.Array,
):
    del B_x
    batch, q_len, d_model = A_x.shape
    _, n_heads, seq, head_dim = A_k_cache.shape
    d_ffn = B_w1.shape[1]
    window = min(4096, max(256, seq // 4))
    n_groups = n_heads // _GROUP
    assert batch == 1 and q_len == 1 and head_dim == _HEAD_DIM
    assert n_heads % _GROUP == 0 and n_groups >= 2 and A_wq.shape[1] == n_heads * head_dim
    assert window % 256 == 0 and (seq - window) % 256 == 0
    assert sum(_W2_ROWS) == d_ffn and d_ffn % _FFN_BLK == 0

    k_t = A_k_cache.reshape(n_heads, seq, head_dim).transpose(0, 2, 1).reshape(n_groups, _GD, seq)
    v_t = A_v_cache.reshape(n_heads, seq, head_dim).transpose(0, 2, 1).reshape(n_groups, _GD, seq)
    dtype = A_x.dtype

    out = pl.pallas_call(
        lambda *refs: _kernel(*refs, window=window),
        out_shape=jax.ShapeDtypeStruct((1, d_model), dtype),
        in_specs=[pl.BlockSpec(memory_space=pl.ANY)] * 8,
        out_specs=pl.BlockSpec((1, d_model), lambda: (0, 0)),
        scratch_shapes=[
            pltpu.VMEM((1, d_model), dtype),
            pltpu.VMEM(A_wq.shape, A_wq.dtype),
            pltpu.VMEM(A_wo.shape, A_wo.dtype),
            pltpu.VMEM((_NSLOT, _GD, window), A_k_cache.dtype),
            pltpu.VMEM((_NSLOT, _GD, window), A_v_cache.dtype),
            pltpu.VMEM(B_w1.shape, B_w1.dtype),
            pltpu.VMEM(B_w3.shape, B_w3.dtype),
            pltpu.VMEM(B_w2.shape, B_w2.dtype),
            pltpu.VMEM((_ROWS, d_ffn), jnp.float32),
            pltpu.SemaphoreType.DMA((_NSEM,)),
        ],
        compiler_params=pltpu.CompilerParams(vmem_limit_bytes=64 * 1024 * 1024),
        name="fused_attn_swiglu_decode",
    )(A_x.reshape(1, d_model), k_t, v_t, A_wq, A_wo, B_w1, B_w3, B_w2)
    return out.reshape(batch, q_len, d_model)
```

```python
import jax
import jax.numpy as jnp
from jax import lax
import jax.experimental.pallas as pl
import jax.experimental.pallas.tpu as pltpu

_EPS = 1e-5
_HEAD_DIM = 192
_GROUP = 2
_GD = _GROUP * _HEAD_DIM
_NSLOT = 2
_ROWS = 8
_FFN_BLK = 384
_W2_ROWS = (512, 512, 384, 128)
_STRIPES = 8

_S_X, _S_A, _S_B, _S_K, _S_V, _NSEM = 0, 1, 2, 3, 5, 7


def _layernorm(x):
    mean = jnp.mean(x, axis=-1, keepdims=True)
    xc = x - mean
    var = jnp.mean(xc * xc, axis=-1, keepdims=True)
    return xc * lax.rsqrt(var + _EPS)


def _start_tile(src, dst, sem, row0, rows, src_col, dst_col, cols, thread):
    pltpu.make_async_copy(
        src.at[pl.ds(row0, rows), pl.ds(src_col, cols)],
        dst.at[pl.ds(row0, rows), pl.ds(dst_col, cols)],
        sem,
    ).start(priority=thread)


def _start_striped(src, dst, sem, tile_rows, tile_cols):
    n_rows, n_cols = dst.shape
    per_stripe = n_rows // (tile_rows * _STRIPES)
    assert per_stripe * tile_rows * _STRIPES == n_rows and n_cols % tile_cols == 0

    def body(i, carry):
        for c in range(0, n_cols, tile_cols):
            for s in range(_STRIPES):
                row0 = pl.multiple_of((s * per_stripe + i) * tile_rows, tile_rows)
                _start_tile(src, dst, sem, row0, tile_rows, c, c, tile_cols, s % 2)
        return carry

    if per_stripe == 1:
        body(0, None)
    else:
        lax.fori_loop(0, per_stripe, body, None)


def _start_window(src, dst, sem, col0):
    n_rows, width = dst.shape
    half = width // 2
    for c in (0, half):
        def body(i, carry, c=c):
            for t in range(2):
                row0 = pl.multiple_of((2 * i + t) * 8, 8)
                _start_tile(src, dst, sem, row0, 8, col0 + c, c, half, t)
            return carry

        lax.fori_loop(0, n_rows // 16, body, None)


def _wait_all(dst, sem):
    pltpu.make_async_copy(dst, dst, sem).wait()


def _kernel(x_hbm, k_hbm, v_hbm, wq_hbm, wo_hbm, w1_hbm, w3_hbm, w2_hbm, o_ref,
            xbuf, wqbuf, wobuf, kbuf, vbuf, w1buf, w3buf, w2buf, act_scr, sems,
            *, window):
    f32, bf16 = jnp.float32, jnp.bfloat16
    n_groups, _, seq = k_hbm.shape
    d_model = xbuf.shape[1]
    d_ffn = w1buf.shape[1]
    col0 = seq - window

    def start_k(j):
        slot = j % _NSLOT
        _start_window(k_hbm.at[j], kbuf.at[slot], sems.at[_S_K + slot], col0)

    def start_v(j):
        slot = j % _NSLOT
        _start_window(v_hbm.at[j], vbuf.at[slot], sems.at[_S_V + slot], col0)

    pltpu.make_async_copy(x_hbm, xbuf, sems.at[_S_X]).start()
    _start_striped(wq_hbm, wqbuf, sems.at[_S_A], 8, 2048)
    _start_striped(wo_hbm, wobuf, sems.at[_S_B], 16, d_model)
    start_k(0)
    start_v(0)
    start_k(1)
    _wait_all(xbuf, sems.at[_S_X])
    _wait_all(wqbuf, sems.at[_S_A])
    _wait_all(wobuf, sems.at[_S_B])

    x = xbuf[...].astype(f32)
    xn = _layernorm(jnp.broadcast_to(x, (_ROWS, d_model))).astype(bf16)

    row = lax.broadcasted_iota(jnp.int32, (_ROWS, _GD), 0)
    col = lax.broadcasted_iota(jnp.int32, (_ROWS, _GD), 1)
    diag = (col >= row * _HEAD_DIM) & (col < (row + 1) * _HEAD_DIM)
    scale = _HEAD_DIM ** -0.5

    def group(j, acc):
        slot = j % _NSLOT
        off = pl.multiple_of(j * _GD, 128)
        q = jnp.dot(xn, wqbuf[:, pl.ds(off, _GD)], preferred_element_type=f32)
        q = jnp.where(diag, q, 0.0).astype(bf16)

        _wait_all(kbuf.at[slot], sems.at[_S_K + slot])

        @pl.when(j + 1 < n_groups)
        def _():
            start_v(j + 1)

        @pl.when(j + 1 == n_groups)
        def _():
            _start_striped(w1_hbm, w1buf, sems.at[_S_A], 8, d_ffn)

        s = jnp.dot(q, kbuf[slot], preferred_element_type=f32) * scale
        p = jnp.exp(s - jnp.max(s, axis=-1, keepdims=True))
        l = jnp.sum(p, axis=-1, keepdims=True)

        _wait_all(vbuf.at[slot], sems.at[_S_V + slot])

        @pl.when(j + 2 < n_groups)
        def _():
            start_k(j + 2)

        @pl.when(j + 1 == n_groups)
        def _():
            _start_striped(w3_hbm, w3buf, sems.at[_S_B], 8, d_ffn)

        o = lax.dot_general(p.astype(bf16), vbuf[slot], (((1,), (1,)), ((), ())),
                            preferred_element_type=f32)
        o = jnp.where(diag, o / l, 0.0).astype(bf16)
        return acc + jnp.dot(o, wobuf[pl.ds(off, _GD), :], preferred_element_type=f32)

    acc = lax.fori_loop(0, n_groups, group, jnp.zeros((_ROWS, d_model), f32))

    w2_chunks = []
    lo = 0
    for c, rows in enumerate(_W2_ROWS):
        sem = sems.at[_S_K + c]
        _start_striped(w2_hbm.at[pl.ds(lo, rows), :], w2buf.at[pl.ds(lo, rows), :],
                       sem, 16, d_model)
        w2_chunks.append((lo, rows, sem))
        lo += rows

    h = x + jnp.sum(acc, axis=0, keepdims=True)
    h = jnp.broadcast_to(h, (_ROWS, d_model))
    hn = _layernorm(h).astype(bf16)

    _wait_all(w1buf, sems.at[_S_A])
    _wait_all(w3buf, sems.at[_S_B])

    def ffn_block(b, carry):
        off = pl.multiple_of(b * _FFN_BLK, 128)
        gate = jnp.dot(hn, w1buf[:, pl.ds(off, _FFN_BLK)], preferred_element_type=f32)
        up = jnp.dot(hn, w3buf[:, pl.ds(off, _FFN_BLK)], preferred_element_type=f32)
        act_scr[:, pl.ds(off, _FFN_BLK)] = gate * jax.nn.sigmoid(gate) * up
        return carry

    lax.fori_loop(0, d_ffn // _FFN_BLK, ffn_block, None)

    out = h
    for lo, rows, sem in w2_chunks:
        act = act_scr[:, lo:lo + rows].astype(bf16)
        _wait_all(w2buf.at[pl.ds(lo, rows), :], sem)
        out = out + jnp.dot(act, w2buf[lo:lo + rows, :], preferred_element_type=f32)
    o_ref[...] = out[0:1, :].astype(o_ref.dtype)


def pallas_sequential_preLN__sliding_block_cached__glu_gated_swiglu__decode_kernel(
    A_x: jax.Array,
    A_k_cache: jax.Array,
    A_v_cache: jax.Array,
    A_wq: jax.Array,
    A_wo: jax.Array,
    B_x: jax.Array,
    B_w1: jax.Array,
    B_w3: jax.Array,
    B_w2: jax.Array,
):
    del B_x
    batch, q_len, d_model = A_x.shape
    _, n_heads, seq, head_dim = A_k_cache.shape
    d_ffn = B_w1.shape[1]
    window = min(4096, max(256, seq // 4))
    n_groups = n_heads // _GROUP
    assert batch == 1 and q_len == 1 and head_dim == _HEAD_DIM
    assert n_heads % _GROUP == 0 and n_groups >= 2 and A_wq.shape[1] == n_heads * head_dim
    assert window % 256 == 0 and (seq - window) % 256 == 0
    assert sum(_W2_ROWS) == d_ffn and d_ffn % _FFN_BLK == 0

    k_t = A_k_cache.reshape(n_heads, seq, head_dim).transpose(0, 2, 1).reshape(n_groups, _GD, seq)
    v_t = A_v_cache.reshape(n_heads, seq, head_dim).transpose(0, 2, 1).reshape(n_groups, _GD, seq)
    dtype = A_x.dtype

    out = pl.pallas_call(
        lambda *refs: _kernel(*refs, window=window),
        out_shape=jax.ShapeDtypeStruct((1, d_model), dtype),
        in_specs=[pl.BlockSpec(memory_space=pl.ANY)] * 8,
        out_specs=pl.BlockSpec((1, d_model), lambda: (0, 0)),
        scratch_shapes=[
            pltpu.VMEM((1, d_model), dtype),
            pltpu.VMEM(A_wq.shape, A_wq.dtype),
            pltpu.VMEM(A_wo.shape, A_wo.dtype),
            pltpu.VMEM((_NSLOT, _GD, window), A_k_cache.dtype),
            pltpu.VMEM((_NSLOT, _GD, window), A_v_cache.dtype),
            pltpu.VMEM(B_w1.shape, B_w1.dtype),
            pltpu.VMEM(B_w3.shape, B_w3.dtype),
            pltpu.VMEM(B_w2.shape, B_w2.dtype),
            pltpu.VMEM((_ROWS, d_ffn), jnp.float32),
            pltpu.SemaphoreType.DMA((_NSEM,)),
        ],
        compiler_params=pltpu.CompilerParams(vmem_limit_bytes=64 * 1024 * 1024),
        name="fused_attn_swiglu_decode",
    )(A_x.reshape(1, d_model), k_t, v_t, A_wq, A_wo, B_w1, B_w3, B_w2)
    return out.reshape(batch, q_len, d_model)
```

```python
import jax
import jax.numpy as jnp
from jax import lax
import jax.experimental.pallas as pl
import jax.experimental.pallas.tpu as pltpu

_EPS = 1e-5
_HEAD_DIM = 192
_GROUP = 2
_GD = _GROUP * _HEAD_DIM
_NSLOT = 2
_ROWS = 8
_FFN_BLK = 512
_W2_ROWS = (512, 384, 384, 256)

_S_X, _S_A, _S_B, _S_K, _S_V, _NSEM = 0, 1, 2, 3, 5, 7


def _layernorm(x):
    mean = jnp.mean(x, axis=-1, keepdims=True)
    xc = x - mean
    var = jnp.mean(xc * xc, axis=-1, keepdims=True)
    return xc * lax.rsqrt(var + _EPS)


def _start_tile(src, dst, sem, row0, rows, src_col, dst_col, cols, thread):
    pltpu.make_async_copy(
        src.at[pl.ds(row0, rows), pl.ds(src_col, cols)],
        dst.at[pl.ds(row0, rows), pl.ds(dst_col, cols)],
        sem,
    ).start(priority=thread)


def _start_striped(src, dst, sem, tile_rows, tile_cols, n_stripes):
    n_rows, n_cols = dst.shape
    per_stripe = n_rows // (tile_rows * n_stripes)
    assert per_stripe * tile_rows * n_stripes == n_rows and n_cols % tile_cols == 0
    assert n_stripes % 2 == 0

    def body(i, carry):
        for c in range(0, n_cols, tile_cols):
            for s in range(n_stripes):
                row0 = pl.multiple_of((s * per_stripe + i) * tile_rows, tile_rows)
                _start_tile(src, dst, sem, row0, tile_rows, c, c, tile_cols, s % 2)
        return carry

    if per_stripe == 1:
        body(0, None)
    else:
        lax.fori_loop(0, per_stripe, body, None)


def _start_window(src, dst, sem, col0):
    n_rows, width = dst.shape
    half = width // 2
    for c in (0, half):
        def body(i, carry, c=c):
            for t in range(2):
                row0 = pl.multiple_of((2 * i + t) * 8, 8)
                _start_tile(src, dst, sem, row0, 8, col0 + c, c, half, t)
            return carry

        lax.fori_loop(0, n_rows // 16, body, None)


def _wait_all(dst, sem):
    pltpu.make_async_copy(dst, dst, sem).wait()


def _kernel(x_hbm, k_hbm, v_hbm, wq_hbm, wo_hbm, w1_hbm, w3_hbm, w2_hbm, o_ref,
            xbuf, wqbuf, wobuf, kbuf, vbuf, w1buf, w3buf, w2buf, act_scr, sems,
            *, window):
    f32, bf16 = jnp.float32, jnp.bfloat16
    n_groups, _, seq = k_hbm.shape
    d_model = xbuf.shape[1]
    d_ffn = w1buf.shape[1]
    col0 = seq - window

    def start_k(j):
        slot = j % _NSLOT
        _start_window(k_hbm.at[j], kbuf.at[slot], sems.at[_S_K + slot], col0)

    def start_v(j):
        slot = j % _NSLOT
        _start_window(v_hbm.at[j], vbuf.at[slot], sems.at[_S_V + slot], col0)

    pltpu.make_async_copy(x_hbm, xbuf, sems.at[_S_X]).start()
    _start_striped(wq_hbm, wqbuf, sems.at[_S_A], 8, 2048, 10)
    _start_striped(wo_hbm, wobuf, sems.at[_S_B], 16, d_model, 8)
    start_k(0)
    start_v(0)
    start_k(1)
    _wait_all(xbuf, sems.at[_S_X])
    _wait_all(wqbuf, sems.at[_S_A])
    _wait_all(wobuf, sems.at[_S_B])

    x = xbuf[...].astype(f32)
    xn = _layernorm(jnp.broadcast_to(x, (_ROWS, d_model))).astype(bf16)

    row = lax.broadcasted_iota(jnp.int32, (_ROWS, _GD), 0)
    col = lax.broadcasted_iota(jnp.int32, (_ROWS, _GD), 1)
    diag = (col >= row * _HEAD_DIM) & (col < (row + 1) * _HEAD_DIM)
    scale = _HEAD_DIM ** -0.5

    def group(j, acc):
        slot = j % _NSLOT
        off = pl.multiple_of(j * _GD, 128)
        q = jnp.dot(xn, wqbuf[:, pl.ds(off, _GD)], preferred_element_type=f32)
        q = jnp.where(diag, q, 0.0).astype(bf16)

        _wait_all(kbuf.at[slot], sems.at[_S_K + slot])

        @pl.when(j + 1 < n_groups)
        def _():
            start_v(j + 1)

        @pl.when(j + 1 == n_groups)
        def _():
            _start_striped(w1_hbm, w1buf, sems.at[_S_A], 8, d_ffn, 8)

        s = jnp.dot(q, kbuf[slot], preferred_element_type=f32) * scale
        p = jnp.exp(s - jnp.max(s, axis=-1, keepdims=True))
        l = jnp.sum(p, axis=-1, keepdims=True)

        _wait_all(vbuf.at[slot], sems.at[_S_V + slot])

        @pl.when(j + 2 < n_groups)
        def _():
            start_k(j + 2)

        @pl.when(j + 1 == n_groups)
        def _():
            _start_striped(w3_hbm, w3buf, sems.at[_S_B], 8, d_ffn, 8)

        o = lax.dot_general(p.astype(bf16), vbuf[slot], (((1,), (1,)), ((), ())),
                            preferred_element_type=f32)
        o = jnp.where(diag, o / l, 0.0).astype(bf16)
        return acc + jnp.dot(o, wobuf[pl.ds(off, _GD), :], preferred_element_type=f32)

    acc = lax.fori_loop(0, n_groups, group, jnp.zeros((_ROWS, d_model), f32))

    w2_chunks = []
    lo = 0
    for c, rows in enumerate(_W2_ROWS):
        sem = sems.at[_S_K + c]
        _start_striped(w2_hbm.at[pl.ds(lo, rows), :], w2buf.at[pl.ds(lo, rows), :],
                       sem, 16, d_model, 4)
        w2_chunks.append((lo, rows, sem))
        lo += rows

    h = x + jnp.sum(acc, axis=0, keepdims=True)
    h = jnp.broadcast_to(h, (_ROWS, d_model))
    hn = _layernorm(h).astype(bf16)

    _wait_all(w1buf, sems.at[_S_A])
    _wait_all(w3buf, sems.at[_S_B])

    def ffn_block(b, carry):
        off = pl.multiple_of(b * _FFN_BLK, 128)
        gate = jnp.dot(hn, w1buf[:, pl.ds(off, _FFN_BLK)], preferred_element_type=f32)
        up = jnp.dot(hn, w3buf[:, pl.ds(off, _FFN_BLK)], preferred_element_type=f32)
        act_scr[:, pl.ds(off, _FFN_BLK)] = gate * jax.nn.sigmoid(gate) * up
        return carry

    lax.fori_loop(0, d_ffn // _FFN_BLK, ffn_block, None)

    out = h
    for lo, rows, sem in w2_chunks:
        act = act_scr[:, lo:lo + rows].astype(bf16)
        _wait_all(w2buf.at[pl.ds(lo, rows), :], sem)
        out = out + jnp.dot(act, w2buf[lo:lo + rows, :], preferred_element_type=f32)
    o_ref[...] = out[0:1, :].astype(o_ref.dtype)


def pallas_sequential_preLN__sliding_block_cached__glu_gated_swiglu__decode_kernel(
    A_x: jax.Array,
    A_k_cache: jax.Array,
    A_v_cache: jax.Array,
    A_wq: jax.Array,
    A_wo: jax.Array,
    B_x: jax.Array,
    B_w1: jax.Array,
    B_w3: jax.Array,
    B_w2: jax.Array,
):
    del B_x
    batch, q_len, d_model = A_x.shape
    _, n_heads, seq, head_dim = A_k_cache.shape
    d_ffn = B_w1.shape[1]
    window = min(4096, max(256, seq // 4))
    n_groups = n_heads // _GROUP
    assert batch == 1 and q_len == 1 and head_dim == _HEAD_DIM
    assert n_heads % _GROUP == 0 and n_groups >= 2 and A_wq.shape[1] == n_heads * head_dim
    assert window % 256 == 0 and (seq - window) % 256 == 0
    assert sum(_W2_ROWS) == d_ffn and d_ffn % _FFN_BLK == 0

    k_t = A_k_cache.reshape(n_heads, seq, head_dim).transpose(0, 2, 1).reshape(n_groups, _GD, seq)
    v_t = A_v_cache.reshape(n_heads, seq, head_dim).transpose(0, 2, 1).reshape(n_groups, _GD, seq)
    dtype = A_x.dtype

    out = pl.pallas_call(
        lambda *refs: _kernel(*refs, window=window),
        out_shape=jax.ShapeDtypeStruct((1, d_model), dtype),
        in_specs=[pl.BlockSpec(memory_space=pl.ANY)] * 8,
        out_specs=pl.BlockSpec((1, d_model), lambda: (0, 0)),
        scratch_shapes=[
            pltpu.VMEM((1, d_model), dtype),
            pltpu.VMEM(A_wq.shape, A_wq.dtype),
            pltpu.VMEM(A_wo.shape, A_wo.dtype),
            pltpu.VMEM((_NSLOT, _GD, window), A_k_cache.dtype),
            pltpu.VMEM((_NSLOT, _GD, window), A_v_cache.dtype),
            pltpu.VMEM(B_w1.shape, B_w1.dtype),
            pltpu.VMEM(B_w3.shape, B_w3.dtype),
            pltpu.VMEM(B_w2.shape, B_w2.dtype),
            pltpu.VMEM((_ROWS, d_ffn), jnp.float32),
            pltpu.SemaphoreType.DMA((_NSEM,)),
        ],
        compiler_params=pltpu.CompilerParams(vmem_limit_bytes=64 * 1024 * 1024),
        name="fused_attn_swiglu_decode",
    )(A_x.reshape(1, d_model), k_t, v_t, A_wq, A_wo, B_w1, B_w3, B_w2)
    return out.reshape(batch, q_len, d_model)
```
